```python
import os as _os
_os.environ.setdefault('JAX_PLATFORMS', 'cpu')
import jax
import jax.numpy as jnp

def _softmax(x, axis=-1):
    return jax.nn.softmax(x, axis=axis)

def _gelu(x):
    return jax.nn.gelu(x, approximate=True)

def _silu(x):
    return jax.nn.silu(x)

def _sigmoid(x):
    return jax.nn.sigmoid(x)

def _layernorm(x, axis=-1, eps=1e-05):
    m = jnp.mean(x, axis=axis, keepdims=True)
    v = jnp.var(x, axis=axis, keepdims=True)
    return (x - m) / jnp.sqrt(v + eps)

def _scatter_add(tgt, idx, src, axis=0):
    return tgt.at[idx].add(src)

def _segment_sum(src, seg, n):
    return jax.ops.segment_sum(src, seg, n)

class _Rng:

    def __init__(self, key):
        self._k = key

    def _next(self):
        self._k, sub = jax.random.split(self._k)
        return sub

    def normal(self, shape):
        return jax.random.normal(self._next(), shape, dtype=jnp.bfloat16)

    def randint(self, lo, hi, shape):
        return jax.random.randint(self._next(), shape, lo, hi, dtype=jnp.int32)

    def uniform(self, shape, lo=0.0, hi=1.0):
        return jax.random.uniform(self._next(), shape, jnp.bfloat16, lo, hi)

    def permutation(self, n):
        return jax.random.permutation(self._next(), n)
kernel_name = 'standalone__conformer_conv_module__speech'

def setup_inputs():
    _rng = _Rng(jax.random.key(int.from_bytes(__import__("os").urandom(4), "little")))
    _w = lambda a: (lambda t: t.astype(jnp.bfloat16) if jnp.issubdtype(t.dtype, jnp.floating) else t)(jnp.asarray(a))
    B, T, D, K = (2, 16000, 256, 5)
    return {'x': _w((lambda *s: _rng.normal(s) * 0.2)(B, T, D)), 'w_pw1': _w((lambda *s: _rng.normal(s) * 0.2)(D, 2 * D)), 'dw': _w((lambda *s: _rng.normal(s) * 0.05)(K, D)), 'w_pw2': _w((lambda *s: _rng.normal(s) * 0.05)(D, D))}

def reference(x, w_pw1, dw, w_pw2):
    B, T, D = x.shape
    K = dw.shape[0]
    h = x @ w_pw1
    a, b = (h[..., :D].copy(), h[..., D:].copy())
    h = a * _sigmoid(b)
    pad = K // 2
    hp = jnp.pad(h, ((0, 0), (pad, pad), (0, 0)))
    out = jnp.zeros_like(h)
    for i in range(K):
        out = out + hp[:, i:i + T, :] * dw[i][None, None, :]
    return _silu(out) @ w_pw2
```

```python
import functools

import jax
import jax.numpy as jnp
import jax.experimental.pallas as pl
import jax.experimental.pallas.tpu as pltpu

HALO = 16
BT = 2000


def _kernel(xp_ref, x_ref, xn_ref, w1_ref, dw_ref, w2_ref, o_ref, h_scr, *, BT, D, K, T):
    i = pl.program_id(1)
    w1 = w1_ref[...] * 0.5
    dw = dw_ref[...].astype(jnp.float32) * 0.5
    xcat = jnp.concatenate([xp_ref[0], x_ref[0], xn_ref[0]], axis=0)
    h = jnp.dot(xcat, w1, preferred_element_type=jnp.float32)
    a = h[:, :D]
    b = h[:, D:]
    g = a * jnp.tanh(b) + a
    rows = jax.lax.broadcasted_iota(jnp.int32, (BT + 2 * HALO, 1), 0) + (i * BT - HALO)
    valid = jnp.logical_and(rows >= 0, rows < T)
    g = jnp.where(valid, g, 0.0)
    h_scr[...] = g
    pad = K // 2
    acc = None
    for k in range(K):
        term = h_scr[pl.ds(HALO - pad + k, BT), :] * dw[k:k + 1, :]
        acc = term if acc is None else acc + term
    s = acc * jnp.tanh(acc) + acc
    o_ref[0] = jnp.dot(
        s.astype(jnp.bfloat16), w2_ref[...], preferred_element_type=jnp.float32
    ).astype(o_ref.dtype)


@jax.jit
def pallas_standalone__conformer_conv_module__speech_kernel(
    x: jax.Array,
    w_pw1: jax.Array,
    dw: jax.Array,
    w_pw2: jax.Array,
):
    B, T, D = x.shape
    K = dw.shape[0]
    assert T % BT == 0 and BT % HALO == 0 and K // 2 <= HALO
    nb = T // BT
    r = BT // HALO
    nh = T // HALO
    kern = functools.partial(_kernel, BT=BT, D=D, K=K, T=T)
    return pl.pallas_call(
        kern,
        grid=(B, nb),
        in_specs=[
            pl.BlockSpec((1, HALO, D), lambda b, i: (b, jnp.maximum(i * r - 1, 0), 0)),
            pl.BlockSpec((1, BT, D), lambda b, i: (b, i, 0)),
            pl.BlockSpec((1, HALO, D), lambda b, i: (b, jnp.minimum((i + 1) * r, nh - 1), 0)),
            pl.BlockSpec((D, 2 * D), lambda b, i: (0, 0)),
            pl.BlockSpec((K, D), lambda b, i: (0, 0)),
            pl.BlockSpec((D, D), lambda b, i: (0, 0)),
        ],
        out_specs=pl.BlockSpec((1, BT, D), lambda b, i: (b, i, 0)),
        out_shape=jax.ShapeDtypeStruct((B, T, D), x.dtype),
        scratch_shapes=[pltpu.VMEM((BT + 2 * HALO, D), jnp.float32)],
        compiler_params=pltpu.CompilerParams(
            dimension_semantics=("parallel", "arbitrary"),
            vmem_limit_bytes=100 * 1024 * 1024,
        ),
    )(x, x, x, w_pw1, dw, w_pw2)
```

```python
import functools

import jax
import jax.numpy as jnp
from jax import lax
import jax.experimental.pallas as pl
import jax.experimental.pallas.tpu as pltpu

HALO = 16
CHUNK = 4000
RAMP = (400, 1200, 2400)


def _kernel(x_hbm, w1_hbm, dw_hbm, w2_hbm, o_hbm,
            x_v, o_v, w1_v, dw_v, w2_v, w1s, dws, h_scr,
            pre_sem, head_sem, tail_sem, out_sem, w_sem, *, B, T, D, K, C, ramp):
    assert B == 2
    NL = D // 128
    S = sum(ramp)
    m = (T - S) // C
    assert S + m * C == T and all(r % HALO == 0 for r in ramp) and C % HALO == 0
    assert K // 2 <= HALO
    NR = len(ramp)
    TP = T + 2 * HALO

    def x_copy(g, bofs, rows, sem):
        return pltpu.make_async_copy(
            x_hbm.at[pl.ds(g, rows), :], x_v.at[pl.ds(g + HALO + bofs, rows), :], sem)

    def o_copy(g, rows):
        return pltpu.make_async_copy(
            o_v.at[pl.ds(g, rows), :], o_hbm.at[pl.ds(g, rows), :], out_sem.at[0])

    def reg(j):
        g = S + j * C
        if isinstance(j, int):
            return g, (2 * HALO if j >= m else 0)
        return pl.multiple_of(g, HALO), jnp.where(j >= m, 2 * HALO, 0)

    def head_copy(j):
        g, bo = reg(j)
        return x_copy(g, bo, HALO, head_sem.at[j % 2])

    def tail_copy(j, size=C):
        g, bo = reg(j)
        return x_copy(g + HALO, bo, size - HALO, tail_sem.at[j % 2])

    ramp_st = [sum(ramp[:r]) for r in range(NR)]

    def pre_copy(r):
        lo = 0 if r == 0 else ramp_st[r] + HALO
        hi = ramp_st[r] + ramp[r] + HALO
        assert hi <= T
        return x_copy(lo, 0, hi - lo, pre_sem.at[r])

    wc = [pltpu.make_async_copy(w1_hbm, w1_v, w_sem.at[0]),
          pltpu.make_async_copy(dw_hbm, dw_v, w_sem.at[0]),
          pltpu.make_async_copy(w2_hbm, w2_v, w_sem.at[0])]
    pre_copy(0).start()
    for w in wc:
        w.start()
    zeros = jnp.zeros((HALO, D), x_v.dtype)
    for b in range(B):
        x_v[b * TP:b * TP + HALO, :] = zeros
        x_v[b * TP + HALO + T:(b + 1) * TP, :] = zeros
    for w in wc:
        w.wait()
    w1s[...] = w1_v[...] * 0.5
    dws[...] = dw_v[...].astype(jnp.float32) * 0.5

    def compute(g, bofs, R):
        xs = g + bofs
        if not isinstance(xs, int):
            xs = pl.multiple_of(xs, HALO)
        xc = x_v[pl.ds(xs, R + 2 * HALO), :]
        h = jnp.dot(xc, w1s[...], preferred_element_type=jnp.float32)
        a = h[:, :D]
        gl = a * jnp.tanh(h[:, D:]) + a
        for l in range(NL):
            h_scr[l, pl.ds(0, R + 2 * HALO), :] = gl[:, l * 128:(l + 1) * 128]
        dw = dws[...]
        pad = K // 2
        cols = []
        for l in range(NL):
            acc = None
            for k in range(K):
                term = (h_scr[l, pl.ds(HALO - pad + k, R), :]
                        * dw[k:k + 1, l * 128:(l + 1) * 128])
                acc = term if acc is None else acc + term
            cols.append(acc)
        acc = jnp.concatenate(cols, axis=1)
        s = acc * jnp.tanh(acc) + acc
        o_v[pl.ds(g, R), :] = jnp.dot(
            s.astype(jnp.bfloat16), w2_v[...],
            preferred_element_type=jnp.float32).astype(o_v.dtype)

    for r in range(NR):
        pre_copy(r).wait()
        if r + 1 < NR:
            pre_copy(r + 1).start()
        else:
            tail_copy(0).start()
            head_copy(1).start()
        compute(ramp_st[r], 0, ramp[r])
        o_copy(ramp_st[r], ramp[r]).start()

    def body(j, carry):
        tail_copy(j).wait()
        head_copy(j + 1).wait()

        @pl.when(j + 1 < 2 * m)
        def _():
            tail_copy(j + 1).start()
            head_copy(j + 2).start()

        @pl.when(j + 1 == 2 * m)
        def _():
            tail_copy(2 * m, S).start()

        g, bo = reg(j)
        compute(g, bo, C)
        o_copy(g, C).start()
        return carry

    lax.fori_loop(0, 2 * m, body, 0)

    tail_copy(2 * m, S).wait()
    down = list(reversed(ramp))
    g = B * T - S
    for r in range(NR):
        compute(g, 2 * HALO, down[r])
        o_copy(g, down[r]).start()
        g += down[r]

    pltpu.make_async_copy(o_v, o_hbm, out_sem.at[0]).wait()


@jax.jit
def pallas_standalone__conformer_conv_module__speech_kernel(
    x: jax.Array,
    w_pw1: jax.Array,
    dw: jax.Array,
    w_pw2: jax.Array,
):
    B, T, D = x.shape
    K = dw.shape[0]
    kern = functools.partial(_kernel, B=B, T=T, D=D, K=K, C=CHUNK, ramp=RAMP)
    any_spec = pl.BlockSpec(memory_space=pl.ANY)
    out = pl.pallas_call(
        kern,
        in_specs=[any_spec] * 4,
        out_specs=any_spec,
        out_shape=jax.ShapeDtypeStruct((B * T, D), x.dtype),
        scratch_shapes=[
            pltpu.VMEM((B * (T + 2 * HALO), D), x.dtype),
            pltpu.VMEM((B * T, D), x.dtype),
            pltpu.VMEM((D, 2 * D), w_pw1.dtype),
            pltpu.VMEM((K, D), dw.dtype),
            pltpu.VMEM((D, D), w_pw2.dtype),
            pltpu.VMEM((D, 2 * D), w_pw1.dtype),
            pltpu.VMEM((K, D), jnp.float32),
            pltpu.VMEM((D // 128, max(CHUNK, max(RAMP)) + 2 * HALO, 128), jnp.float32),
            pltpu.SemaphoreType.DMA((len(RAMP),)),
            pltpu.SemaphoreType.DMA((2,)),
            pltpu.SemaphoreType.DMA((2,)),
            pltpu.SemaphoreType.DMA((1,)),
            pltpu.SemaphoreType.DMA((1,)),
        ],
        compiler_params=pltpu.CompilerParams(
            vmem_limit_bytes=110 * 1024 * 1024,
        ),
    )(x.reshape(B * T, D), w_pw1, dw, w_pw2)
    return out.reshape(B, T, D)
```

```python
import functools

import jax
import jax.numpy as jnp
from jax import lax
import jax.experimental.pallas as pl
import jax.experimental.pallas.tpu as pltpu

HALO = 16

UP = (560, 1200, 2240)
GA = (4400,)
GB = (4000, 2400, 1200)
DOWN = (2080, 1120, 480, 240, 80)


def _kernel(x_hbm, w1_hbm, dw_hbm, w2_hbm, o_hbm,
            x_v, o_v, w1_v, dw_v, w2_v, w1s, dws, h_scr,
            pre_sem, a_sem, b_sem, out_sem, w_sem, *, B, T, D, K, up, ga, gb, down):
    assert B == 2
    NL = D // 128
    S = sum(up)
    LA, LB = sum(ga), sum(gb)
    L = LA + LB
    assert sum(down) == S and S + L == T and K // 2 <= HALO
    assert all(r % HALO == 0 for r in up + down + ga + gb)
    NU = len(up)
    TP = T + HALO

    def x_copy(g, bofs, rows, sem):
        return pltpu.make_async_copy(
            x_hbm.at[pl.ds(g, rows), :], x_v.at[pl.ds(g + bofs, rows), :], sem)

    def o_copy(g, rows):
        return pltpu.make_async_copy(
            o_v.at[pl.ds(g, rows), :], o_hbm.at[pl.ds(g, rows), :], out_sem.at[0])

    def base(j):
        if isinstance(j, int):
            return S + j * L, HALO * j
        return pl.multiple_of(S + j * L, HALO), pl.multiple_of(HALO * j, HALO)

    def a_copies(j):
        g, bo = base(j)
        return [x_copy(g + HALO, bo, LA, a_sem.at[0])]

    def b_copies(j):
        g, bo = base(j)
        return [x_copy(g + LA + HALO, bo, LB - HALO, b_sem.at[0]),
                x_copy(g + L, HALO, HALO, b_sem.at[0])]

    def d_copy():
        return x_copy(2 * T - S + HALO, HALO, S - HALO, a_sem.at[0])

    up_st = [sum(up[:r]) for r in range(NU)]

    def pre_copy(r):
        lo = 0 if r == 0 else up_st[r] + HALO
        hi = up_st[r] + up[r] + HALO
        assert hi <= T
        return x_copy(lo, 0, hi - lo, pre_sem.at[r])

    wc = [pltpu.make_async_copy(w1_hbm, w1_v, w_sem.at[0]),
          pltpu.make_async_copy(dw_hbm, dw_v, w_sem.at[0]),
          pltpu.make_async_copy(w2_hbm, w2_v, w_sem.at[0])]
    pre_copy(0).start()
    for w in wc:
        w.start()
    zeros = jnp.zeros((HALO, D), x_v.dtype)
    for b in range(B):
        x_v[b * TP + T:(b + 1) * TP, :] = zeros
    for l in range(NL):
        h_scr[l, 0:HALO, :] = jnp.zeros((HALO, 128), jnp.float32)
    for w in wc:
        w.wait()
    w1s[...] = w1_v[...] * 0.5
    dws[...] = dw_v[...].astype(jnp.float32) * 0.5

    def compute(g, bofs, R, lo, skip):
        xs = g + bofs + skip
        if not isinstance(xs, int):
            xs = pl.multiple_of(xs, HALO)
            g = pl.multiple_of(g, HALO)
        n = R + HALO - skip
        xc = x_v[pl.ds(xs, n), :]
        h = jnp.dot(xc, w1s[...], preferred_element_type=jnp.float32)
        a = h[:, :D]
        gl = a * jnp.tanh(h[:, D:]) + a
        for l in range(NL):
            h_scr[l, pl.ds(lo + HALO + skip, n), :] = gl[:, l * 128:(l + 1) * 128]
        dw = dws[...]
        pad = K // 2
        cols = []
        for l in range(NL):
            acc = None
            for k in range(K):
                term = (h_scr[l, pl.ds(lo + HALO - pad + k, R), :]
                        * dw[k:k + 1, l * 128:(l + 1) * 128])
                acc = term if acc is None else acc + term
            cols.append(acc)
        acc = jnp.concatenate(cols, axis=1)
        s = acc * jnp.tanh(acc) + acc
        o_v[pl.ds(g, R), :] = jnp.dot(
            s.astype(jnp.bfloat16), w2_v[...],
            preferred_element_type=jnp.float32).astype(o_v.dtype)
        o_copy(g, R).start()

    def carry(src, rows, keep=None):
        for l in range(NL):
            v = h_scr[l, pl.ds(src, rows), :]
            if keep is not None:
                v = jnp.where(keep, v, 0.0)
            h_scr[l, pl.ds(0, rows), :] = v

    for r in range(NU):
        pre_copy(r).wait()
        if r + 1 < NU:
            pre_copy(r + 1).start()
        else:
            for c in a_copies(0):
                c.start()
        compute(up_st[r], 0, up[r], up_st[r], 0 if r == 0 else HALO)
    carry(S, HALO)

    def body(j, c_):
        g, bo = base(j)
        for c in a_copies(j):
            c.wait()
        for c in b_copies(j):
            c.start()
        lo = 0
        for i, R in enumerate(ga):
            compute(g + lo, bo, R, lo, 0 if i == 0 else HALO)
            lo += R
        for c in b_copies(j):
            c.wait()

        @pl.when(j == 0)
        def _():
            for c in a_copies(1):
                c.start()

        @pl.when(j == 1)
        def _():
            d_copy().start()

        for R in gb:
            compute(g + lo, bo, R, lo, HALO)
            lo += R
        carry(L, 2 * HALO, keep=(j != 0))
        return c_

    lax.fori_loop(0, 2, body, 0)

    d_copy().wait()
    g = B * T - S
    lo = 0
    for R in down:
        compute(g, HALO, R, lo, HALO)
        g += R
        lo += R

    pltpu.make_async_copy(o_v, o_hbm, out_sem.at[0]).wait()


@jax.jit
def pallas_standalone__conformer_conv_module__speech_kernel(
    x: jax.Array,
    w_pw1: jax.Array,
    dw: jax.Array,
    w_pw2: jax.Array,
):
    B, T, D = x.shape
    K = dw.shape[0]
    kern = functools.partial(
        _kernel, B=B, T=T, D=D, K=K, up=UP, ga=GA, gb=GB, down=DOWN)
    any_spec = pl.BlockSpec(memory_space=pl.ANY)
    h_rows = max(sum(GA) + sum(GB), sum(UP)) + 2 * HALO
    out = pl.pallas_call(
        kern,
        in_specs=[any_spec] * 4,
        out_specs=any_spec,
        out_shape=jax.ShapeDtypeStruct((B * T, D), x.dtype),
        scratch_shapes=[
            pltpu.VMEM((B * (T + HALO), D), x.dtype),
            pltpu.VMEM((B * T, D), x.dtype),
            pltpu.VMEM((D, 2 * D), w_pw1.dtype),
            pltpu.VMEM((K, D), dw.dtype),
            pltpu.VMEM((D, D), w_pw2.dtype),
            pltpu.VMEM((D, 2 * D), w_pw1.dtype),
            pltpu.VMEM((K, D), jnp.float32),
            pltpu.VMEM((D // 128, h_rows, 128), jnp.float32),
            pltpu.SemaphoreType.DMA((len(UP),)),
            pltpu.SemaphoreType.DMA((1,)),
            pltpu.SemaphoreType.DMA((1,)),
            pltpu.SemaphoreType.DMA((1,)),
            pltpu.SemaphoreType.DMA((1,)),
        ],
        compiler_params=pltpu.CompilerParams(
            vmem_limit_bytes=110 * 1024 * 1024,
        ),
    )(x.reshape(B * T, D), w_pw1, dw, w_pw2)
    return out.reshape(B, T, D)
```

```python
import functools

import jax
import jax.numpy as jnp
from jax import lax
import jax.experimental.pallas as pl
import jax.experimental.pallas.tpu as pltpu

HALO = 16

UP = (560, 1200, 2240)
GA = (4400,)
GB = (4000, 2400, 1200)
DOWN = (2080, 1120, 480, 240, 80)


def _kernel(x_hbm, w1_hbm, dw_hbm, w2_hbm, o_hbm,
            x_v, o_v, w1_v, dw_v, w2_v, dws, h_scr,
            x_sem, out_sem, w_sem, *, B, T, D, K, up, ga, gb, down):
    assert B == 2
    NL = D // 128
    S = sum(up)
    LA, LB = sum(ga), sum(gb)
    L = LA + LB
    assert sum(down) == S and S + L == T and K // 2 <= HALO
    assert all(r % HALO == 0 for r in up + down + ga + gb)
    NU = len(up)
    TP = T + HALO

    def x_copy(g, bofs, rows):
        return pltpu.make_async_copy(
            x_hbm.at[pl.ds(g, rows), :], x_v.at[pl.ds(g + bofs, rows), :], x_sem.at[0])

    def o_copy(g, rows):
        return pltpu.make_async_copy(
            o_v.at[pl.ds(g, rows), :], o_hbm.at[pl.ds(g, rows), :], out_sem.at[0])

    def base(j):
        if isinstance(j, int):
            return S + j * L, HALO * j
        return pl.multiple_of(S + j * L, HALO), pl.multiple_of(HALO * j, HALO)

    def a_copies(j):
        g, bo = base(j)
        return [x_copy(g + HALO, bo, LA)]

    def b_copies(j):
        g, bo = base(j)
        return [x_copy(g + LA + HALO, bo, LB - HALO), x_copy(g + L, HALO, HALO)]

    def d_copy():
        return x_copy(2 * T - S + HALO, HALO, S - HALO)

    up_st = [sum(up[:r]) for r in range(NU)]

    def pre_copy(r):
        lo = 0 if r == 0 else up_st[r] + HALO
        hi = up_st[r] + up[r] + HALO
        assert hi <= T
        return x_copy(lo, 0, hi - lo)

    wc = [pltpu.make_async_copy(w1_hbm, w1_v, w_sem.at[0]),
          pltpu.make_async_copy(dw_hbm, dw_v, w_sem.at[0]),
          pltpu.make_async_copy(w2_hbm, w2_v, w_sem.at[0])]
    pre_copy(0).start()
    for w in wc:
        w.start()
    zeros = jnp.zeros((HALO, D), x_v.dtype)
    for b in range(B):
        x_v[b * TP + T:(b + 1) * TP, :] = zeros
    for l in range(NL):
        h_scr[l, 0:HALO, :] = jnp.zeros((HALO, 128), jnp.float32)
    for w in wc:
        w.wait()
    dws[...] = dw_v[...].astype(jnp.float32) * 0.25

    def compute(g, bofs, R, lo, skip):
        xs = g + bofs + skip
        if not isinstance(xs, int):
            xs = pl.multiple_of(xs, HALO)
            g = pl.multiple_of(g, HALO)
        n = R + HALO - skip
        xc = x_v[pl.ds(xs, n), :]
        h = jnp.dot(xc, w1_v[...], preferred_element_type=jnp.float32)
        a = h[:, :D]
        gl = a * jnp.tanh(h[:, D:] * 0.5) + a
        for l in range(NL):
            h_scr[l, pl.ds(lo + HALO + skip, n), :] = gl[:, l * 128:(l + 1) * 128]
        dw = dws[...]
        pad = K // 2
        cols = []
        for l in range(NL):
            acc = None
            for k in range(K):
                term = (h_scr[l, pl.ds(lo + HALO - pad + k, R), :]
                        * dw[k:k + 1, l * 128:(l + 1) * 128])
                acc = term if acc is None else acc + term
            cols.append(acc)
        acc = jnp.concatenate(cols, axis=1)
        s = acc * jnp.tanh(acc) + acc
        o_v[pl.ds(g, R), :] = jnp.dot(
            s.astype(jnp.bfloat16), w2_v[...],
            preferred_element_type=jnp.float32).astype(o_v.dtype)
        o_copy(g, R).start()

    def carry(src, rows, keep=None):
        for l in range(NL):
            v = h_scr[l, pl.ds(src, rows), :]
            if keep is not None:
                v = jnp.where(keep, v, 0.0)
            h_scr[l, pl.ds(0, rows), :] = v

    for r in range(NU):
        pre_copy(r).wait()
        if r + 1 < NU:
            pre_copy(r + 1).start()
        else:
            for c in a_copies(0):
                c.start()
        compute(up_st[r], 0, up[r], up_st[r], 0 if r == 0 else HALO)
    carry(S, HALO)

    def body(j, c_):
        g, bo = base(j)
        for c in a_copies(j):
            c.wait()
        for c in b_copies(j):
            c.start()
        lo = 0
        for i, R in enumerate(ga):
            compute(g + lo, bo, R, lo, 0 if i == 0 else HALO)
            lo += R
        for c in b_copies(j):
            c.wait()

        @pl.when(j == 0)
        def _():
            for c in a_copies(1):
                c.start()

        @pl.when(j == 1)
        def _():
            d_copy().start()

        for R in gb:
            compute(g + lo, bo, R, lo, HALO)
            lo += R
        carry(L, 2 * HALO, keep=(j != 0))
        return c_

    lax.fori_loop(0, 2, body, 0)

    d_copy().wait()
    g = B * T - S
    lo = 0
    for R in down:
        compute(g, HALO, R, lo, HALO)
        g += R
        lo += R

    pltpu.make_async_copy(o_v, o_hbm, out_sem.at[0]).wait()


@jax.jit
def pallas_standalone__conformer_conv_module__speech_kernel(
    x: jax.Array,
    w_pw1: jax.Array,
    dw: jax.Array,
    w_pw2: jax.Array,
):
    B, T, D = x.shape
    K = dw.shape[0]
    kern = functools.partial(
        _kernel, B=B, T=T, D=D, K=K, up=UP, ga=GA, gb=GB, down=DOWN)
    any_spec = pl.BlockSpec(memory_space=pl.ANY)
    h_rows = max(sum(GA) + sum(GB), sum(UP)) + 2 * HALO
    out = pl.pallas_call(
        kern,
        in_specs=[any_spec] * 4,
        out_specs=any_spec,
        out_shape=jax.ShapeDtypeStruct((B * T, D), x.dtype),
        scratch_shapes=[
            pltpu.VMEM((B * (T + HALO), D), x.dtype),
            pltpu.VMEM((B * T, D), x.dtype),
            pltpu.VMEM((D, 2 * D), w_pw1.dtype),
            pltpu.VMEM((K, D), dw.dtype),
            pltpu.VMEM((D, D), w_pw2.dtype),
            pltpu.VMEM((K, D), jnp.float32),
            pltpu.VMEM((D // 128, h_rows, 128), jnp.float32),
            pltpu.SemaphoreType.DMA((1,)),
            pltpu.SemaphoreType.DMA((1,)),
            pltpu.SemaphoreType.DMA((1,)),
        ],
        compiler_params=pltpu.CompilerParams(
            vmem_limit_bytes=110 * 1024 * 1024,
        ),
    )(x.reshape(B * T, D), w_pw1, dw, w_pw2)
    return out.reshape(B, T, D)
```
